```python
import jax
import jax.numpy as jnp

def _softmax(x, axis=-1):
    return jax.nn.softmax(x, axis=axis)
def _gelu(x):
    return jax.nn.gelu(x, approximate=True)
def _silu(x):
    return jax.nn.silu(x)
def _sigmoid(x):
    return jax.nn.sigmoid(x)
def _layernorm(x, axis=-1, eps=1e-5):
    m = jnp.mean(x, axis=axis, keepdims=True)
    v = jnp.var(x, axis=axis, keepdims=True)
    return (x - m) / jnp.sqrt(v + eps)
def _scatter_add(tgt, idx, src, axis=0):
    return tgt.at[idx].add(src)
def _segment_sum(src, seg, n):
    return jax.ops.segment_sum(src, seg, n)
class _Rng:
    def __init__(self, key):
        self._k = key
    def _next(self):
        self._k, sub = jax.random.split(self._k)
        return sub
    def normal(self, shape):
        return jax.random.normal(self._next(), shape, dtype=jnp.bfloat16)
    def randint(self, lo, hi, shape):
        return jax.random.randint(self._next(), shape, lo, hi, dtype=jnp.int32)
    def uniform(self, shape, lo=0.0, hi=1.0):
        return jax.random.uniform(self._next(), shape, jnp.bfloat16, lo, hi)
    def permutation(self, n):
        return jax.random.permutation(self._next(), n)


kernel_name = 'standalone__convnext_block__vision'

def setup_inputs():
    _rng = _Rng(jax.random.key(int.from_bytes(__import__("os").urandom(4), "little")))
    _w = (lambda a: (lambda t: t.astype(jnp.bfloat16) if jnp.issubdtype(t.dtype, jnp.floating) else t)(jnp.asarray(a)))
    H = W = 512
    C = 96
    return {
        "x": _w((lambda *s: _rng.normal(s) * 0.05)(1, H, W, C)),
        "dw": _w((lambda *s: _rng.normal(s) * 0.05)(7, 7, C)),
        "w1": _w((lambda *s: _rng.normal(s) * 0.05)(C, 4 * C)),
        "w2": _w((lambda *s: _rng.normal(s) * 0.05)(4 * C, C)),
    }

def reference(x, dw, w1, w2):
    B, H, W, C = x.shape
    pad = 3
    xp = jnp.pad(x, ((0,0),(pad,pad),(pad,pad),(0,0)))
    out = jnp.zeros_like(x)
    for i in range(7):
        for j in range(7):
            out = out + xp[:, i:i+H, j:j+W, :] * dw[i, j][None, None, None, :]
    h = _layernorm(out, axis=-1)
    return x + _gelu(h @ w1) @ w2
```

```python
import functools
import numpy as np
import jax
import jax.numpy as jnp
from jax import lax
import jax.experimental.pallas as pl
import jax.experimental.pallas.tpu as pltpu

F32, BF16, U32 = jnp.float32, jnp.bfloat16, jnp.uint32
_C1 = float(np.sqrt(2.0 / np.pi))
_C2 = _C1 * 0.044715
_ALPHA = float(np.cbrt(_C2))

G = 16
PITCH = 97
LAG = 20
OG = 8
NSEM = 4


def _kernel(x_hbm, dw_ref, w1_ref, w2t_ref, o_hbm,
            xbuf, cbuf, carry, amat, w1t, obuf, isem, osem, *, H, W, C, unroll):
    NT = W // 128
    CP = C // 2
    NG = H // G
    PPC = CP // G

    def in_copy(g, k):
        rows = pl.ds(pl.multiple_of(g * (G * CP), G * CP), G * CP)
        return pltpu.make_async_copy(
            x_hbm.bitcast(U32).at[rows, pl.ds(k * 128, 128)], xbuf.at[k, rows, :],
            isem.at[g % NSEM, k])

    def out_copy(q):
        rows = pl.ds(pl.multiple_of(q * (OG * C), OG * C), OG * C)
        return pltpu.make_async_copy(obuf.at[q % 2], o_hbm.at[rows, :], osem.at[q % 2])

    for g in range(2):
        for k in range(NT):
            in_copy(g, k).start()

    w1 = jnp.concatenate([w1_ref[...].astype(F32), jnp.zeros((128 - C, 4 * C), F32)], axis=0)
    w1t[...] = pltpu.bitcast(w1.T.astype(BF16), U32)

    lane = lax.broadcasted_iota(jnp.int32, (C, 128), 1)
    kj = lane // 16
    krow = (lane % 16) // 2 + 8 * (lane % 2)
    d = []
    for i in range(7):
        dwi = jnp.concatenate([dw_ref[i].astype(F32), jnp.zeros((1, C), F32)], axis=0)
        dwi = jnp.concatenate([dwi, jnp.zeros((8, 128 - C), F32)], axis=1)
        dwi = jnp.concatenate([dwi, jnp.zeros((120, 128), F32)], axis=0).T[:C]
        acc = jnp.zeros((C, 128), F32)
        for j in range(7):
            acc = jnp.where(kj == j, dwi[:, j:j + 1], acc)
        d.append(acc)

    def build(rho, _):
        acc = jnp.zeros((C, 128), F32)
        tap = krow - rho + 7
        for i in range(7):
            acc = jnp.where(tap == i, d[i], acc)
        amat[pl.ds(rho, C, stride=24), :] = acc
    lax.fori_loop(0, 24, build, None)
    carry[...] = jnp.zeros(carry.shape, F32)

    wl = lax.broadcasted_iota(jnp.int32, (8, 128), 1)

    def shifted(v, dlt):
        if dlt == 0:
            return v
        r = [pltpu.roll(t, (-dlt) % 128, 1) for t in v]
        z = jnp.zeros((8, 128), U32)
        if dlt > 0:
            m = wl < 128 - dlt
            return [jnp.where(m, r[k], r[k + 1] if k + 1 < NT else z) for k in range(NT)]
        m = wl >= -dlt
        return [jnp.where(m, r[k], r[k - 1] if k > 0 else z) for k in range(NT)]

    def conv_chunk(t):
        g = t // G
        p0 = (t % G) * PPC
        pos = (g % 2) * G
        for pp in range(PPC):
            p = p0 + pp
            lo, hi = [], []
            for k in range(NT):
                a = xbuf[k, pl.ds(g * (G * CP) + p, 8, stride=CP), :]
                b = xbuf[k, pl.ds(g * (G * CP) + 8 * CP + p, 8, stride=CP), :]
                lo.append((a & jnp.uint32(0xFFFF)) | (b << 16))
                hi.append((a >> 16) | (b & jnp.uint32(0xFFFF0000)))
            for u, v in enumerate((lo, hi)):
                c = 2 * p + u
                rhs = jnp.concatenate(
                    [jnp.concatenate(shifted(v, j - 3), axis=1) for j in range(7)], axis=0)
                rhs = pltpu.bitcast(rhs, BF16)
                lhs = amat[pl.ds(pl.multiple_of(c * 24, 8), 24), :][:, :112]
                o = lax.dot_general(lhs, rhs, (((1,), (0,)), ((), ())),
                                    preferred_element_type=F32)
                o0 = o[0:8] + carry[c]
                carry[c] = o[16:24]
                for k in range(NT):
                    cbuf[k, pl.ds(pos * PITCH + c, 8, stride=PITCH), :] = o0[:, k * 128:(k + 1) * 128]
                    cbuf[k, pl.ds((pos + 8) * PITCH + c, 8, stride=PITCH), :] = o[8:16, k * 128:(k + 1) * 128]

    def mlp_row(h):
        pos = (h + 4) % (2 * G)
        y = jnp.concatenate([cbuf[k, pl.ds(pos * PITCH, C), :] for k in range(NT)], axis=1)
        mean = jnp.sum(y, axis=0, keepdims=True) * (1.0 / C)
        yc = y - mean
        var = jnp.sum(yc * yc, axis=0, keepdims=True) * (1.0 / C)
        hn = (yc * (lax.rsqrt(var + 1e-5) * _ALPHA)).astype(BF16)
        z = jnp.dot(pltpu.bitcast(w1t[...], BF16)[:, :C], hn, preferred_element_type=F32)
        th = jnp.tanh(z * (z * z + _C1 / _ALPHA))
        gl = (z * th + z).astype(BF16)
        o = jnp.dot(w2t_ref[...], gl, preferred_element_type=F32)
        rows = pl.ds(pl.multiple_of(h * CP, CP), CP)
        xr = pltpu.bitcast(jnp.concatenate([xbuf[k, rows, :] for k in range(NT)], axis=1), BF16).astype(F32)
        res = (xr + o * (0.5 / _ALPHA)).astype(BF16)
        obuf[(h // OG) % 2, pl.ds(pl.multiple_of((h % OG) * C, C), C), :] = res

    def in_sync(t):
        @pl.when(t % G == 0)
        def _():
            g = t // G
            for k in range(NT):
                in_copy(g, k).wait()

            @pl.when(g + 2 < NG)
            def _():
                for k in range(NT):
                    in_copy(g + 2, k).start()

    def out_pre(h):
        @pl.when(jnp.logical_and(h % OG == 0, h >= 2 * OG))
        def _():
            out_copy(h // OG - 2).wait()

    def out_post(h):
        @pl.when(h % OG == OG - 1)
        def _():
            out_copy(h // OG).start()

    def pro(t, _):
        in_sync(t)
        conv_chunk(t)
    lax.fori_loop(0, LAG, pro, None)

    def main(i, _):
        t = LAG + i * unroll
        in_sync(t)
        out_pre(t - LAG)
        for u in range(unroll):
            mlp_row(t + u - LAG)
            conv_chunk(t + u)
        out_post(t + unroll - 1 - LAG)
    lax.fori_loop(0, (H - LAG) // unroll, main, None)

    def flush(c, _):
        v = carry[c]
        for k in range(NT):
            cbuf[k, pl.ds((NG % 2) * G * PITCH + c, 8, stride=PITCH), :] = v[:, k * 128:(k + 1) * 128]
    lax.fori_loop(0, C, flush, None)

    def epi(h, _):
        out_pre(h)
        mlp_row(h)
        out_post(h)
    lax.fori_loop(H - LAG, H, epi, None)
    out_copy(H // OG - 2).wait()
    out_copy(H // OG - 1).wait()


def make(unroll=1):
    @jax.jit
    def pallas_standalone__convnext_block__vision_kernel(x, dw, w1, w2):
        B, H, W, C = x.shape
        x2 = jnp.transpose(x, (0, 1, 3, 2)).reshape(H * C, W)
        NT = W // 128
        out = pl.pallas_call(
            functools.partial(_kernel, H=H, W=W, C=C, unroll=unroll),
            out_shape=jax.ShapeDtypeStruct((H * C, W), x.dtype),
            in_specs=[pl.BlockSpec(memory_space=pl.ANY),
                      pl.BlockSpec(memory_space=pltpu.VMEM),
                      pl.BlockSpec(memory_space=pltpu.VMEM),
                      pl.BlockSpec(memory_space=pltpu.VMEM)],
            out_specs=pl.BlockSpec(memory_space=pl.ANY),
            scratch_shapes=[
                pltpu.VMEM((NT, H * C // 2, 128), U32),
                pltpu.VMEM((NT, 2 * G * PITCH, 128), F32),
                pltpu.VMEM((C, 8, W), F32),
                pltpu.VMEM((C * 24, 128), F32),
                pltpu.VMEM((2 * C, 128), U32),
                pltpu.VMEM((2, OG * C, W), BF16),
                pltpu.SemaphoreType.DMA((NSEM, NT)),
                pltpu.SemaphoreType.DMA((2,)),
            ],
            compiler_params=pltpu.CompilerParams(vmem_limit_bytes=100 * 1024 * 1024),
            name="convnext",
        )(x2, dw, w1, w2.T)
        return jnp.transpose(out.reshape(B, H, C, W), (0, 1, 3, 2))
    return pallas_standalone__convnext_block__vision_kernel


pallas_standalone__convnext_block__vision_kernel = make(unroll=1)
```

```python
import functools
import numpy as np
import jax
import jax.numpy as jnp
from jax import lax
import jax.experimental.pallas as pl
import jax.experimental.pallas.tpu as pltpu

F32, BF16, U32 = jnp.float32, jnp.bfloat16, jnp.uint32
_C1 = float(np.sqrt(2.0 / np.pi))
_C2 = _C1 * 0.044715
_ALPHA = float(np.cbrt(_C2))

G = 16
PITCH = 97
RP = 9
NSEM = 4
OG = 8


def _pack(a, b):
    return pltpu.pack_elementwise([a, b], packed_dtype=BF16)


def _unpack(v):
    return [pltpu.unpack_elementwise(v, index=i, packed_dtype=BF16, unpacked_dtype=F32) for i in range(2)]


def _kernel(x_hbm, dw_ref, w1_ref, w2t_ref, o_hbm,
            xbuf, rbuf, cbuf, carry, amat, w1t, w2t, b0, b1, b2, b3, zref, isem, osem,
            *, H, W, C, U, order, m1c, alloc, opaque, fast, j3):
    NT = W // 128
    CP = C // 2
    NG = H // G
    CPC = C // G
    bufs = [b0, b1, b2, b3]
    S0, H0, G0, O0 = 0, 336, 336 + 96, 336 + 96 + 384
    sbuf, hbuf, gbuf, obuf = [bufs[int(a)] for a in alloc]
    zref[0] = 0

    def z8(name):
        return pl.multiple_of(zref[0], 8) if name in opaque else 0

    def rd(buf, r0, n):
        return jnp.concatenate([buf[k, r0:r0 + n, :] for k in range(NT)], axis=1)

    def in_copy(g, k):
        rows = pl.ds(pl.multiple_of(g * (G * CP), G * CP), G * CP)
        return pltpu.make_async_copy(
            x_hbm.bitcast(U32).at[rows, pl.ds(k * 128, 128)], xbuf.at[k, rows, :],
            isem.at[g & (NSEM - 1), k])

    def out_copy(q, k):
        rows = pl.ds(pl.multiple_of(q * (OG * CP), OG * CP), OG * CP)
        src = pl.ds(pl.multiple_of(O0 + (q & 1) * (OG * CP), 8), OG * CP)
        return pltpu.make_async_copy(
            obuf.at[k, src, :], o_hbm.bitcast(U32).at[rows, pl.ds(k * 128, 128)], osem.at[q & 1, k])

    def in_start(g):
        for k in range(NT):
            in_copy(g, k).start()

    def in_wait(g):
        for k in range(NT):
            in_copy(g, k).wait()

    in_start(0)

    def prep():
        w1 = jnp.concatenate([w1_ref[...].astype(F32), jnp.zeros((128 - C, 4 * C), F32)], axis=0)
        ev, od = _unpack(pltpu.bitcast(w1.T.astype(BF16), U32))
        hc = m1c // 2
        w1t[...] = pltpu.bitcast(jnp.concatenate(
            [v[i:i + hc] for i in range(0, 2 * C, hc) for v in (ev, od)], axis=0).astype(BF16), U32)
        w2t[...] = pltpu.bitcast(jnp.concatenate(_unpack(pltpu.bitcast(w2t_ref[...], U32)), axis=0).astype(BF16), U32)

        lane = lax.broadcasted_iota(jnp.int32, (C, 128), 1)
        kj = lane >> 4
        krow = lane & 15
        d = []
        for i in range(7):
            dwi = jnp.concatenate([dw_ref[i].astype(F32), jnp.zeros((1, C), F32)], axis=0)
            dwi = jnp.concatenate([dwi, jnp.zeros((8, 128 - C), F32)], axis=1)
            dwi = jnp.concatenate([dwi, jnp.zeros((120, 128), F32)], axis=0).T[:C]
            acc = jnp.zeros((C, 128), F32)
            for j in range(7):
                acc = jnp.where(kj == j, dwi[:, j:j + 1], acc)
            d.append(acc)

        def build(rho, _):
            acc = jnp.zeros((C, 128), F32)
            tap = krow - rho + 7
            for i in range(7):
                acc = jnp.where(tap == i, d[i], acc)
            amat[pl.ds(rho, C, stride=24), :] = acc
        lax.fori_loop(0, 24, build, None)
        carry[...] = jnp.zeros(carry.shape, F32)
    if not fast:
        prep()

    wl = lax.broadcasted_iota(jnp.int32, (8, 128), 1)

    def shifted(v, dlt):
        if dlt == 0:
            return v
        r = [pltpu.roll(t, (-dlt) % 128, 1) for t in v]
        z = jnp.zeros((8, 128), U32)
        if dlt > 0:
            m = wl < 128 - dlt
            return [jnp.where(m, r[k], r[k + 1] if k + 1 < NT else z) for k in range(NT)]
        m = wl >= -dlt
        return [jnp.where(m, r[k], r[k - 1] if k > 0 else z) for k in range(NT)]

    def cpos(t, i):
        return (t & 15) * (CPC // 2) + (i // 2 + CP * (i % 2))

    def relayout(p, k):
        a = xbuf[k, pl.ds(pl.multiple_of(p * C, 8), CP), :]
        b = xbuf[k, pl.ds(pl.multiple_of(p * C + CP, 8), CP), :]
        base = ((p >> 3) & 3) * (C * RP) + (p & 7)
        rbuf[k, pl.ds(base, CP, stride=RP), :] = (a & jnp.uint32(0xFFFF)) | (b << 16)
        rbuf[k, pl.ds(base + CP * RP, CP, stride=RP), :] = (a >> 16) | (b & jnp.uint32(0xFFFF0000))

    def rload(t, i):
        base = ((t >> 4) & 3) * (C * RP) + cpos(t, i) * RP
        return [rbuf[k, pl.ds(base, 8), :] for k in range(NT)]

    def shift_ch(t, i):
        v = rload(t, i)
        z = z8("s")
        for j in range(7):
            if j == 3 and j3:
                continue
            for k, tl in enumerate(shifted(v, j - 3)):
                sbuf[k, pl.ds(z + S0 + 56 * i + 8 * j, 8), :] = tl

    def conv_mm(t, i):
        c = (t & 15) * CPC + i
        lhs = amat[pl.ds(pl.multiple_of(c * 24, 8), 24), :][:, :112]
        if j3:
            rhs = jnp.concatenate([rd(sbuf, S0 + 56 * i, 24), jnp.concatenate(rload(t, i), axis=1),
                                   rd(sbuf, S0 + 56 * i + 32, 24)], axis=0)
        else:
            rhs = rd(sbuf, S0 + 56 * i, 56)
        return lax.dot_general(lhs, pltpu.bitcast(rhs, BF16), (((1,), (0,)), ((), ())), preferred_element_type=F32)

    def conv_fin(t, i, o):
        c = cpos(t, i)
        pos = (t & 48) * PITCH + c
        o0 = o[0:8] + carry[c]
        carry[c] = o[16:24]
        for k in range(NT):
            cbuf[k][pl.ds(pos, 8, stride=PITCH), :] = o0[:, k * 128:(k + 1) * 128]
            cbuf[k][pl.ds(pos + 8 * PITCH, 8, stride=PITCH), :] = o[8:16, k * 128:(k + 1) * 128]

    def ln(h, k, slot):
        pos = (h + 4) & (4 * G - 1)
        y = cbuf[k][pl.ds(pos * PITCH, C), :]
        mean = jnp.sum(y, axis=0, keepdims=True) * (1.0 / C)
        yc = y - mean
        var = jnp.sum(yc * yc, axis=0, keepdims=True) * (1.0 / C)
        hn = yc * (lax.rsqrt(var + 1e-5) * _ALPHA)
        hbuf[k, pl.ds(z8("h") + H0 + slot * CP, CP), :] = _pack(hn[:CP], hn[CP:])

    def mm1(i, slot):
        r0, r1 = i * m1c // 2, (i + 1) * m1c // 2
        return jnp.dot(pltpu.bitcast(w1t[r0:r1, :], BF16)[:, :C], pltpu.bitcast(rd(hbuf, H0 + slot * CP, CP), BF16),
                       preferred_element_type=F32)

    def gelu(i, slot, z):
        th = jnp.tanh(z * (z * z + _C1 / _ALPHA))
        gl = z * th + z
        p = _pack(gl[:m1c // 2], gl[m1c // 2:])
        zz = z8("g")
        for k in range(NT):
            gbuf[k, pl.ds(zz + G0 + slot * 2 * C + i * m1c // 2, m1c // 2), :] = p[:, k * 128:(k + 1) * 128]

    def mm2(i, slot):
        return jnp.dot(pltpu.bitcast(w2t[:, i * 128:(i + 1) * 128], BF16),
                       pltpu.bitcast(rd(gbuf, G0 + slot * 2 * C + i * 64, 64), BF16), preferred_element_type=F32)

    def fin(h, k, o):
        rows = pl.ds(pl.multiple_of(h * CP, CP), CP)
        dst = pl.ds(pl.multiple_of(O0 + (h & (2 * OG - 1)) * CP, 8), CP)
        xe, xo = _unpack(xbuf[k, rows, :])
        ok = o[:, k * 128:(k + 1) * 128] * (0.5 / _ALPHA)
        obuf[k, dst, :] = _pack(xe + ok[:CP], xo + ok[CP:])

    def steps(t0, n, par0, en):
        toks = order.split()
        has = lambda o: any(x.lstrip("-")[0] == o for x in toks)
        st = [dict() for _ in range(n)]

        def run(tok, u):
            t, par = t0 + u, (par0 + u) & 1
            op = tok[0]
            for i in ([int(ch, 16) for ch in tok[1:]]):
                if op == "L" and "L" in en:
                    ln(t - 22, i, 1 - par)
                elif op == "r" and "r" in en:
                    relayout(jnp.minimum((t + 18) >> 1, H // 2 - 1), 2 * par + i)
                elif op == "c" and "c" in en:
                    st[u]["c", i] = conv_mm(t, i)
                    if not has("d"):
                        conv_fin(t, i, st[u]["c", i])
                elif op == "d" and "c" in en:
                    conv_fin(t, i, st[u]["c", i])
                elif op == "s" and "s" in en:
                    shift_ch(t + 1, i)
                elif op == "a" and "a" in en:
                    st[u]["a", i] = mm1(i, par)
                    if not has("g"):
                        gelu(i, par, st[u]["a", i])
                elif op == "g" and "a" in en:
                    gelu(i, par, st[u]["a", i])
                elif op == "b" and "b" in en:
                    o = mm2(i, 1 - par)
                    st[u]["b"] = o if i == 0 else st[u]["b"] + o
                elif op == "f" and "b" in en:
                    fin(t - 24, i, st[u]["b"])

        for u in range(n + 1):
            for tok in toks:
                if tok[0] == "-":
                    if u > 0:
                        run(tok[1:], u - 1)
                elif u < n:
                    run(tok, u)

    in_start(1)
    in_start(2)
    in_wait(0)
    if not fast:
        def rl(p, _):
            for k in range(NT):
                relayout(p, k)
        lax.fori_loop(0, 8, rl, None)
        for i in range(CPC):
            shift_ch(0, i)
        lax.fori_loop(0, 7, lambda i, _: steps(2 * i, 2, 0, "sc"), None)
    in_wait(1)
    in_wait(2)
    in_start(3)
    if not fast:
        lax.fori_loop(8, 21, rl, None)
        lax.fori_loop(7, 11, lambda i, _: steps(2 * i, 2, 0, "sc"), None)
        steps(22, 1, 0, "scL")
        steps(23, 1, 1, "scLa")

    def block(q, en):
        @pl.when(q >= 2)
        def _():
            for k in range(NT):
                out_copy(q - 2, k).wait()
        lax.fori_loop(0, OG // U, lambda i, _: steps(24 + q * OG + i * U, U, 0, en), None)
        for k in range(NT):
            out_copy(q, k).start()

    def main(q, _):
        @pl.when((q & 1) == 0)
        def _():
            g = (q >> 1) + 3
            @pl.when(g < NG)
            def _():
                in_wait(g)
            @pl.when(g + 1 < NG)
            def _():
                in_start(g + 1)
        block(q, "rscLab")
    NQ = H // OG
    lax.fori_loop(0, NQ - 3, main, None)

    def flush(c, _):
        v = carry[c]
        for k in range(NT):
            cbuf[k][pl.ds((NG % 4) * G * PITCH + c, 8, stride=PITCH), :] = v[:, k * 128:(k + 1) * 128]
    lax.fori_loop(0, C, flush, None)

    if not fast:
        lax.fori_loop(NQ - 3, NQ, lambda q, _: block(q, "Lab"), None)
    for q in (NQ - 2, NQ - 1):
        for k in range(NT):
            out_copy(q, k).wait()


def make(U=4, order="r01 L0123 b0 c0 b1 c1 s01 b2 f0123 c2 a0 c3 s23 a1 c4 a2 c5 s45", m1c=128,
         alloc="0123", opaque="", flags=None, fast=False, j3=True):
    @jax.jit
    def pallas_standalone__convnext_block__vision_kernel(x, dw, w1, w2):
        B, H, W, C = x.shape
        x2 = jnp.transpose(x, (0, 1, 3, 2)).reshape(H * C, W)
        NT = W // 128
        out = pl.pallas_call(
            functools.partial(_kernel, H=H, W=W, C=C, U=U, order=order, m1c=m1c, alloc=alloc,
                              opaque=opaque, fast=fast, j3=j3),
            out_shape=jax.ShapeDtypeStruct((H * C, W), x.dtype),
            in_specs=[pl.BlockSpec(memory_space=pl.ANY),
                      pl.BlockSpec(memory_space=pltpu.VMEM),
                      pl.BlockSpec(memory_space=pltpu.VMEM),
                      pl.BlockSpec(memory_space=pltpu.VMEM)],
            out_specs=pl.BlockSpec(memory_space=pl.ANY),
            scratch_shapes=[
                pltpu.VMEM((NT, H * C // 2, 128), U32),
                pltpu.VMEM((NT, 4 * C * RP, 128), U32),
                [pltpu.VMEM((4 * G * PITCH, 128), F32)] * NT,
                pltpu.VMEM((C, 8, W), F32),
                pltpu.VMEM((C * 24, 128), F32),
                pltpu.VMEM((2 * C, 128), U32),
                pltpu.VMEM((C // 2, 4 * C), U32),
                *[pltpu.VMEM((NT, 336 + 96 + 384 + 768, 128), U32)] * 4,
                pltpu.SMEM((1,), jnp.int32),
                pltpu.SemaphoreType.DMA((NSEM, NT)),
                pltpu.SemaphoreType.DMA((2, NT)),
            ],
            compiler_params=pltpu.CompilerParams(vmem_limit_bytes=110 * 1024 * 1024, flags=flags),
            name="convnext",
        )(x2, dw, w1, w2.T)
        return jnp.transpose(out.reshape(B, H, C, W), (0, 1, 3, 2))
    return pallas_standalone__convnext_block__vision_kernel


pallas_standalone__convnext_block__vision_kernel = make(U=8)
```

```python
import functools
import numpy as np
import jax
import jax.numpy as jnp
from jax import lax
import jax.experimental.pallas as pl
import jax.experimental.pallas.tpu as pltpu

F32, BF16, U32 = jnp.float32, jnp.bfloat16, jnp.uint32
_C1 = float(np.sqrt(2.0 / np.pi))
_C2 = _C1 * 0.044715
_ALPHA = float(np.cbrt(_C2))

G = 16
CPITCH = 97
RPITCH = 9
XSLOTS = 8
CSLOT = 1568


def _kernel(x_hbm, dw_hbm, w1_hbm, w2t_hbm, o_hbm,
            xbuf, rbuf, cbuf, carry, obuf, amat, w1t, w2t, sbuf, hbuf, gbuf, dwv, w1v, w2v, isem, osem, wsem,
            *, H, W, C, U, order, m1c, fast, LL):
    NT = W // 128
    CP = C // 2
    NG = H // G
    CPC = C // G
    NA = 4 * C // m1c
    T0 = LL + 2

    def in_copy(g):
        src = jnp.minimum(g, NG - 1) * (G * C)
        dst = (g & (XSLOTS - 1)) * (G * C)
        return pltpu.make_async_copy(
            x_hbm.at[pl.ds(pl.multiple_of(src, G * C), G * C)],
            xbuf.at[pl.ds(pl.multiple_of(dst, G * C), G * C)], isem.at[g & (XSLOTS - 1)])

    def out_copy(r0, n):
        rows = pl.ds(pl.multiple_of(r0 * C, C), n * C)
        return pltpu.make_async_copy(obuf.at[rows], o_hbm.at[rows], osem)

    wcopies = [pltpu.make_async_copy(s, d, wsem.at[i])
               for i, (s, d) in enumerate(((dw_hbm, dwv), (w1_hbm, w1v), (w2t_hbm, w2v)))]
    for cp in wcopies:
        cp.start()
    in_copy(0).start()
    for cp in wcopies:
        cp.wait()

    def prep():
        w1 = jnp.concatenate([w1v[...].astype(F32), jnp.zeros((128 - C, 4 * C), F32)], axis=0)
        w1t[...] = pltpu.bitcast(w1.T.astype(BF16), U32)
        w2t[...] = pltpu.bitcast(w2v[...], U32)

        lane = lax.broadcasted_iota(jnp.int32, (C, 128), 1)
        krow = lane & 15
        spread = (lax.broadcasted_iota(jnp.int32, (128, 128), 0)
                  == (lax.broadcasted_iota(jnp.int32, (128, 128), 1) >> 4)).astype(F32)
        d = []
        for i in range(7):
            dwi = jnp.concatenate([dwv[i].astype(F32), jnp.zeros((1, C), F32)], axis=0)
            dwi = jnp.concatenate([dwi, jnp.zeros((8, 128 - C), F32)], axis=1)
            dwi = jnp.concatenate([dwi, jnp.zeros((120, 128), F32)], axis=0).T[:C]
            d.append(jnp.dot(dwi, spread, preferred_element_type=F32))

        def build(rho, _):
            acc = jnp.zeros((C, 128), F32)
            tap = krow - rho + 7
            for i in range(7):
                acc = jnp.where(tap == i, d[i], acc)
            amat[pl.ds(rho, C, stride=24), :] = acc
        lax.fori_loop(0, 24, build, None)

    wl = lax.broadcasted_iota(jnp.int32, (8, 128), 1)

    def shifted(v, dlt):
        if dlt == 0:
            return v
        r = [pltpu.roll(t, (-dlt) % 128, 1) for t in v]
        z = jnp.zeros((8, 128), U32)
        if dlt > 0:
            m = wl < 128 - dlt
            return [jnp.where(m, r[k], r[k + 1] if k + 1 < NT else z) for k in range(NT)]
        m = wl >= -dlt
        return [jnp.where(m, r[k], r[k - 1] if k > 0 else z) for k in range(NT)]

    def slot(g, n, size):
        v = (g & (n - 1)) * size
        return v if isinstance(v, int) else pl.multiple_of(v, size & -size)

    def xrow(q, f):
        return pl.ds(slot(q + (f >> 4), XSLOTS, G * C) + (f & 15) * C, C)

    def relayout(q, f, k):
        lanes = slice(k * 128, (k + 1) * 128)
        a = pltpu.bitcast(xbuf[xrow(q, f), lanes], U32)
        b = pltpu.bitcast(xbuf[xrow(q, f + 1), lanes], U32)
        base = slot(q + (f >> 4), 4, C * RPITCH) + ((f & 15) >> 1)
        rbuf[k, pl.ds(base, CP, stride=RPITCH), :] = (a & jnp.uint32(0xFFFF)) | (b << 16)
        rbuf[k, pl.ds(base + CP * RPITCH, CP, stride=RPITCH), :] = (a >> 16) | (b & jnp.uint32(0xFFFF0000))

    def shift_ch(q, f, i):
        c = (f & 15) * CPC + i
        base = slot(q + (f >> 4), 4, C * RPITCH) + (c // 2 + CP * (c % 2)) * RPITCH
        v = [rbuf[k, pl.ds(base, 8), :] for k in range(NT)]
        return jnp.concatenate([jnp.concatenate(shifted(v, j - 3), axis=1) for j in range(7)], axis=0)

    def conv_mm(f, i, rhs):
        c = (f & 15) * CPC + i
        return lax.dot_general(amat[c * 24:(c + 1) * 24, :][:, :7 * G], pltpu.bitcast(rhs, BF16),
                               (((1,), (0,)), ((), ())), preferred_element_type=F32)

    def conv_fin(q, f, i, o):
        g = q + (f >> 4)
        c = (f & 15) * CPC + i
        cur = slot(g, 4, CSLOT) + c
        o0 = o[0:8] if isinstance(g, int) and g == 0 else o[0:8] + carry[c]
        carry[c] = o[16:24]
        for k in range(NT):
            cbuf[k][pl.ds(cur, 8, stride=CPITCH), :] = o0[:, k * 128:(k + 1) * 128]
            cbuf[k][pl.ds(cur + 8 * CPITCH, 8, stride=CPITCH), :] = o[8:16, k * 128:(k + 1) * 128]

    def flush(f, i):
        c = (f & 15) * CPC + i
        for k in range(NT):
            cbuf[k][pl.ds(slot(NG, 4, CSLOT) + c, 8, stride=CPITCH), :] = carry[c, :, k * 128:(k + 1) * 128]

    def ln(q, f, k):
        f = f + 4
        y = cbuf[k][pl.ds(slot(q + (f >> 4), 4, CSLOT) + (f & 15) * CPITCH, C), :]
        mean = jnp.sum(y, axis=0, keepdims=True) * (1.0 / C)
        yc = y - mean
        var = jnp.sum(yc * yc, axis=0, keepdims=True) * (1.0 / C)
        return yc * (lax.rsqrt(var + 1e-5) * _ALPHA)

    def mm1(i, h):
        lhs = pltpu.bitcast(w1t[i * m1c // 2:(i + 1) * m1c // 2, :], BF16)[:, :C]
        return lax.dot_general(lhs, h, (((1,), (0,)), ((), ())), preferred_element_type=F32)

    def gelu(z):
        return z * jnp.tanh(z * (z * z + _C1 / _ALPHA)) + z

    def mm2(i, g):
        return lax.dot_general(pltpu.bitcast(w2t[:, i * 128:(i + 1) * 128], BF16), g, (((1,), (0,)), ((), ())), preferred_element_type=F32)

    def fin(q, f, k, o):
        lanes = slice(k * 256, (k + 1) * 256)
        res = xbuf[xrow(q, f), lanes].astype(F32) + o * (0.5 / _ALPHA)
        obuf[pl.ds(slot(q + (f >> 4), NG, G * C) + (f & 15) * C, C), lanes] = res.astype(BF16)

    def put(buf, v):
        if buf.dtype == U32:
            buf.bitcast(BF16)[...] = v.astype(BF16)
        else:
            buf[...] = v.astype(buf.dtype)

    def get(bufs):
        v = jnp.concatenate([b[...] for b in bufs], axis=1)
        return pltpu.bitcast(v, BF16) if v.dtype == U32 else v

    def steps(q, f0, ens):
        n = len(ens)
        toks = order.split()
        st = [dict() for _ in range(n + 1)]

        def run(tok, u):
            f, en, op = f0 + u, ens[u], tok[0]
            for i in ([int(ch, 16) for ch in tok[1:]]):
                if op == "r" and "r" in en:
                    relayout(q, (f + 17) & ~1, 2 * ((f + 17) & 1) + i)
                elif op == "s" and "s" in en:
                    sbuf[i] = shift_ch(q, f + 1, i)
                elif op == "c" and "c" in en:
                    st[u]["c", i] = conv_mm(f, i, sbuf[i])
                elif op == "d" and "c" in en:
                    conv_fin(q, f, i, st[u]["c", i])
                elif op == "d" and "F" in en:
                    flush(f, i)
                elif op == "L" and "L" in en:
                    hbuf.bitcast(BF16)[pl.ds(((f + 1) & 1) * C, C), pl.ds(i * 128, 128)] = ln(q, f - LL, i).astype(BF16)
                elif op == "a" and "a" in en:
                    h = pltpu.bitcast(hbuf[pl.ds((f & 1) * CP, CP), pl.ds(i * 128, 128)], BF16)
                    if m1c == 384:
                        st[u]["a", i] = mm1(0, h)
                    else:
                        st[u]["a", i] = jnp.concatenate([mm1(j, h) for j in range(4)], axis=0)
                elif op == "g" and "a" in en:
                    gbuf.bitcast(BF16)[pl.ds(((f + 1) & 1) * 4 * C, 4 * C), pl.ds(i * 128, 128)] = gelu(st[u]["a", i]).astype(BF16)
                elif op == "b" and "b" in en:
                    t = [mm2(j, pltpu.bitcast(gbuf[pl.ds((f & 1) * 2 * C + j * 64, 64), i * 128:(i + 1) * 128], BF16)) for j in range(3)]
                    st[u]["o", i] = t[0] + t[1] + t[2]
                    o = mm2(i, pltpu.bitcast(gbuf[pl.ds((f & 1) * 2 * C + i * 64, 64), 384:], BF16))
                    st[u]["o", 3] = o if i == 0 else st[u]["o", 3] + o
                elif op == "f" and "b" in en:
                    fin(q, f - LL - 2, i, jnp.concatenate([st[u]["o", 2 * i], st[u]["o", 2 * i + 1]], axis=1))

        for u in range(n + 1):
            for tok in toks:
                if tok[0] == "-":
                    if u > 0:
                        run(tok[1:], u - 1)
                elif u < n:
                    run(tok, u)

    if not fast:
        prep()
    in_copy(1).start()
    in_copy(0).wait()
    in_copy(2).start()
    if not fast:
        steps(0, -17, ["r"] * 16 + ["s"] + ["sc"] * 7)
    in_copy(1).wait()
    in_copy(3).start()
    if not fast:
        steps(0, -1, ["r"] * 8)
        steps(0, 7, ["rsc"] * 8)
    in_copy(2).wait()
    if not fast:
        steps(0, 15, ["rsc"] * (LL - 15) + ["rscL", "rscLa"] + ["rscLab"] * (31 - T0))
    out_copy(0, 31 - T0).start()

    def main(q, _):
        in_copy(q + 2).wait()
        in_copy(q + 3).start()
        steps(q, 15, ["rscLab"] * U)
        out_copy(q * G + 15 - T0, G).start()
    lax.fori_loop(1, NG - 1, main, None)
    in_copy(NG + 1).wait()

    if not fast:
        steps(NG - 1, 15, ["cLab"] + ["FLab"] * 16 + ["Lab"] * (T0 - 19))
    out_copy(H - 1 - T0, T0 - 2).start()
    if not fast:
        steps(NG, T0 - 3, ["Lab", "ab", "b"])
    out_copy(H - 3, 3).start()
    pltpu.make_async_copy(obuf, o_hbm, osem).wait()


ORDER = "-g2 c0 d0 s0 a0 c1 d1 g0 a1 g1 c2 s1 s2 b0 d2 L0 r0 r1 L2 c3 L1 d3 L3 b1 c4 s3 s4 b2 d4 f0 a2 c5 d5 f1 s5"


def make(U=16, order=ORDER, m1c=128, flags=None, fast=False, LL=21, mode="vv", interpret=False, **cp):
    @jax.jit
    def pallas_standalone__convnext_block__vision_kernel(x, dw, w1, w2):
        B, H, W, C = x.shape
        x2 = jnp.transpose(x, (0, 1, 3, 2)).reshape(H * C, W)
        NT = W // 128
        mk = lambda m, n: {"v": pltpu.VMEM((n // 2, 128), U32), "f": pltpu.VMEM((n, 128), F32), "b": pltpu.VMEM((n, 128), BF16)}[m]
        out = pl.pallas_call(
            functools.partial(_kernel, H=H, W=W, C=C, U=U, order=order, m1c=m1c, fast=fast, LL=LL),
            out_shape=jax.ShapeDtypeStruct((H * C, W), x.dtype),
            in_specs=[pl.BlockSpec(memory_space=pl.ANY)] * 4,
            out_specs=pl.BlockSpec(memory_space=pl.ANY),
            scratch_shapes=[
                pltpu.VMEM((XSLOTS * G * C, W), BF16),
                pltpu.VMEM((NT, 4 * C * RPITCH, 128), U32),
                [pltpu.VMEM((4 * CSLOT, 128), F32)] * NT,
                pltpu.VMEM((C, 8, W), F32),
                pltpu.VMEM((H * C, W), BF16),
                pltpu.VMEM((C * 24, 128), F32),
                pltpu.VMEM((2 * C, 128), U32),
                pltpu.VMEM((C // 2, 4 * C), U32),
                pltpu.VMEM((C // G, 56, W), U32),
                pltpu.VMEM((C, W), U32),
                pltpu.VMEM((4 * C, W), U32),
                pltpu.VMEM(dw.shape, BF16),
                pltpu.VMEM(w1.shape, BF16),
                pltpu.VMEM(w1.shape, BF16),
                pltpu.SemaphoreType.DMA((XSLOTS,)),
                pltpu.SemaphoreType.DMA(()),
                pltpu.SemaphoreType.DMA((3,)),
            ],
            compiler_params=pltpu.CompilerParams(vmem_limit_bytes=110 * 1024 * 1024, flags=flags, **cp),
            interpret=interpret,
            name="convnext",
        )(x2, dw, w1, w2.T)
        return jnp.transpose(out.reshape(B, H, C, W), (0, 1, 3, 2))
    return pallas_standalone__convnext_block__vision_kernel


pallas_standalone__convnext_block__vision_kernel = make(m1c=96, order='b0 r0 r1 a0 g0 -d5 c0 a1 s0 -s2 g1 d0 c1 s1 b1 d1 L1 c2 a2 g2 L2 d2 c3 s3 b2 f0 f1 d3 c4 s4 a3 g3 L0 L3 d4 c5 s5')
```

```python
import functools

import numpy as np
import jax
import jax.numpy as jnp
from jax import lax
import jax.experimental.pallas as pl
import jax.experimental.pallas.tpu as pltpu

F32, BF16, U32 = jnp.float32, jnp.bfloat16, jnp.uint32

_C1 = float(np.sqrt(2.0 / np.pi))
_ALPHA = float(np.cbrt(_C1 * 0.044715))
_EPS = 1e-5

LANES = 128
KS = 7
G = 16
GOUT = G + 8
XSLOTS = 8
RSLOTS = 4
RPITCH = 9
LAG = 21
EARLY = (16, 17, 18, 20, 21, 23, 25, 26, 28, 30)

ORDER = ("b0 c0 L0 a0 L1 a1 -d5 -s2 L2 -d4 c1 s1 s0 b1 c2 d0 -s5 r1 r0 -s3 d1 L3 a2 c3 b2 c4 d2 "
         "-f0 s4 c5 g2 d3 a3 g0 g3 g1 f1")
ORDER_FILL = "r0 r1 c0 s0 d0 c1 s1 d1 c2 s2 d2 c3 s3 d3 c4 s4 d4 c5 s5 d5"
ORDER_DRAIN = ORDER


def _dot(a, b):
    return lax.dot_general(a, b, (((1,), (0,)), ((), ())), preferred_element_type=F32)


def _slot(g, n, size):
    v = (g & (n - 1)) * size
    return v if isinstance(v, int) else pl.multiple_of(v, size & -size)


def _tile(k, n=LANES):
    return slice(k * n, (k + 1) * n)


def _kernel(x_hbm, dw_hbm, w1_hbm, w2t_hbm, o_hbm,
            xbuf, rbuf, sbuf, amat, carry, cbuf, gbuf, obuf, w1t, w2t, dwv, w1v, w2v,
            xsem, x0sem, osem, wsem):
    H, C, W = x_hbm.shape
    NT, NG, CP, CPC = W // LANES, H // G, C // 2, C // G
    CPITCH = C + 1
    CSLOT = (cbuf[0].shape[0] - C) // RSLOTS

    def x_copy(g):
        return pltpu.make_async_copy(
            x_hbm.at[pl.ds(jnp.minimum(g, NG - 1) * G, G)],
            xbuf.at[pl.ds(_slot(g, XSLOTS, G), G)], xsem.at[g & (XSLOTS - 1)])

    def x0_copy(m):
        return pltpu.make_async_copy(
            x_hbm.at[0:G, _tile(m, 16)], xbuf.at[0:G, _tile(m, 16)], x0sem.at[m])

    def out_copy(h, n):
        return pltpu.make_async_copy(obuf.at[pl.ds(h, n)], o_hbm.at[pl.ds(h, n)], osem)

    def prepare_weights():
        w1 = jnp.concatenate([w1v[...].astype(F32), jnp.zeros((LANES - C, 4 * C), F32)], axis=0)
        w1t[...] = pltpu.bitcast(w1.T.astype(BF16), U32)
        w2t[...] = pltpu.bitcast(w2v[...], U32)

        spread = jnp.where(lax.broadcasted_iota(jnp.int32, (LANES, LANES), 0)
                           == (lax.broadcasted_iota(jnp.int32, (LANES, LANES), 1) >> 4), 1.0, 0.0)
        taps = []
        for i in range(KS):
            d = jnp.concatenate([dwv[i].astype(F32), jnp.zeros((8 - KS, C), F32)], axis=0)
            d = jnp.concatenate([d, jnp.zeros((8, LANES - C), F32)], axis=1)
            d = jnp.concatenate([d, jnp.zeros((LANES - 8, LANES), F32)], axis=0).T[:C]
            taps.append(_dot(d, spread))
        r = lax.broadcasted_iota(jnp.int32, (C, LANES), 1) & (G - 1)

        def row(rho, _):
            acc = jnp.zeros((C, LANES), F32)
            for i in range(KS):
                acc = jnp.where(r - rho + 7 == i, taps[i], acc)
            amat[pl.ds(rho, C, stride=GOUT), :] = acc
        lax.fori_loop(0, GOUT, row, None)

    def xrow(q, f):
        return _slot(q + (f >> 4), XSLOTS, G) + (f & 15)

    def relayout(q, f, k, c0=0, nc=C):
        a = pltpu.bitcast(xbuf[xrow(q, f), c0:c0 + nc, _tile(k)], U32)
        b = pltpu.bitcast(xbuf[xrow(q, f + 1), c0:c0 + nc, _tile(k)], U32)
        base = _slot(q + (f >> 4), RSLOTS, C * RPITCH) + (c0 // 2 * RPITCH + ((f & 15) >> 1))
        even = (a & np.uint32(0xFFFF)) | (b << 16)
        odd = (a >> 16) | (b & np.uint32(0xFFFF0000))
        rbuf[k, pl.ds(base, nc // 2, stride=RPITCH), :] = even
        rbuf[k, pl.ds(base + CP * RPITCH, nc // 2, stride=RPITCH), :] = odd

    lane = lax.broadcasted_iota(jnp.int32, (8, LANES), 1)

    def shifted(v, d):
        if d == 0:
            return v
        zero = [jnp.zeros((8, LANES), U32)]
        r = [pltpu.roll(t, (-d) % LANES, 1) for t in v]
        own, other = (lane < LANES - d, r[1:] + zero) if d > 0 else (lane >= -d, zero + r[:-1])
        return [jnp.where(own, a, b) for a, b in zip(r, other)]

    def shift(q, f, i):
        c = (f & 15) * CPC + i
        base = _slot(q + (f >> 4), RSLOTS, C * RPITCH) + (c // 2 + CP * (c % 2)) * RPITCH
        v = [rbuf[k, pl.ds(base, 8), :] for k in range(NT)]
        sbuf[i] = jnp.concatenate(
            [jnp.concatenate(shifted(v, j - KS // 2), axis=1) for j in range(KS)], axis=0)

    def conv(f, i):
        c = (f & 15) * CPC + i
        return _dot(amat[_tile(c, GOUT), :][:, :KS * G], pltpu.bitcast(sbuf[i], BF16))

    def conv_store(q, f, i, o):
        g, c = q + (f >> 4), (f & 15) * CPC + i
        if o is None:
            parts = [carry[c]]
        else:
            top = isinstance(g, int) and g == 0
            parts = [o[0:8] if top else o[0:8] + carry[c], o[8:16]]
            carry[c] = o[16:24]
        for k in range(NT):
            for n, p in enumerate(parts):
                rows = pl.ds(_slot(g, RSLOTS, CSLOT) + (8 * n * CPITCH + c), 8, stride=CPITCH)
                cbuf[k][rows, :] = p[:, _tile(k)]

    def layernorm(q, f, k):
        p = f + 4
        y = cbuf[k][pl.ds(_slot(q + (p >> 4), RSLOTS, CSLOT) + (p & 15) * CPITCH, C), :]
        yc = y - jnp.sum(y, axis=0, keepdims=True) * (1.0 / C)
        var = jnp.sum(yc * yc, axis=0, keepdims=True) * (1.0 / C)
        return (yc * (lax.rsqrt(var + _EPS) * _ALPHA)).astype(BF16)

    def expand(h):
        return jnp.concatenate(
            [_dot(pltpu.bitcast(w1t[_tile(j, CP), :], BF16)[:, :C], h) for j in range(4)], axis=0)

    def gelu(f, k, z):
        gbuf[k, _tile(f & 1, 4 * C), :] = z * jnp.tanh(z * (z * z + _C1 / _ALPHA)) + z

    def project(f, k, j):
        g = gbuf[k, pl.ds((f & 1) * 4 * C + j * LANES, LANES), :]
        return _dot(pltpu.bitcast(w2t[:, _tile(j)], BF16), g)

    def residual(q, f, k, o):
        res = xbuf[xrow(q, f), :, _tile(k, 2 * LANES)].astype(F32) + o * (0.5 / _ALPHA)
        obuf[q * G + f, :, _tile(k, 2 * LANES)] = res.astype(BF16)

    def run(q, steps, order):
        vals = [dict() for _ in steps]

        def piece(op, i, st, v):
            if op == "r" and "r" in st:
                relayout(q, st["r"] & ~1, 2 * (st["r"] & 1) + i)
            elif op == "s" and "s" in st:
                shift(q, st["s"], i)
            elif op == "c" and "c" in st:
                v["c", i] = conv(st["c"], i)
            elif op == "d" and "d" in st:
                conv_store(q, st["d"], i, v.get(("c", i)))
            elif op == "L" and "a" in st:
                v["h", i] = layernorm(q, st["a"], i)
            elif op == "a" and "a" in st:
                v["a", i] = expand(v["h", i])
            elif op == "g" and "a" in st:
                gelu(st["a"], i, v["a", i])
            elif op == "b" and "b" in st:
                v["o", i] = project(st["b"], i, 0) + project(st["b"], i, 1) + project(st["b"], i, 2)
                last = project(st["b"], NT - 1, i)
                v["o", NT - 1] = last if i == 0 else v["o", NT - 1] + last
            elif op == "f" and "b" in st:
                residual(q, st["b"], i, jnp.concatenate([v["o", 2 * i], v["o", 2 * i + 1]], axis=1))

        for u in range(len(steps) + 1):
            if u < len(steps):
                for fn in steps[u].get("pre", ()):
                    fn()
            for tok in order.split():
                n = u - 1 if tok[0] == "-" else u
                if 0 <= n < len(steps):
                    piece(tok[-2], int(tok[-1]), steps[n], vals[n])

    def full_step(f):
        return dict(r=f + G + 1, s=f + 1, c=f, d=f, a=f - LAG, b=f - LAG - 1)

    wcopies = [pltpu.make_async_copy(s, d, wsem.at[i])
               for i, (s, d) in enumerate(((dw_hbm, dwv), (w1_hbm, w1v), (w2t_hbm, w2v)))]
    for cp in wcopies:
        cp.start()
    for m in range(C // 16):
        x0_copy(m).start()
    for cp in wcopies:
        cp.wait()
    x_copy(1).start()
    prepare_weights()

    def first_group(m):
        x0_copy(m).wait()
        for f in range(0, G, 2):
            for k in range(NT):
                relayout(0, f, k, 16 * m, 16)

    fill = [dict(s=0)] + [dict(s=f + 1, c=f, d=f) for f in range(2 * G - 1)]

    def before(f, *fns):
        fill[f + 1].setdefault("pre", []).extend(fns)

    for m in range(C // 16):
        before(max(16 * m // CPC - 2, -1), functools.partial(first_group, m))
    before(2, x_copy(2).start)
    before(6, x_copy(1).wait, x_copy(3).start)
    before(G - 1, x_copy(2).wait)
    for n in range(G // 2):
        before(6 + n, *[functools.partial(relayout, 0, G + 2 * n, k) for k in range(NT)])
    for f in range(G - 1, 2 * G - 1):
        fill[f + 1]["r"] = full_step(f)["r"]
    assert len(EARLY) == 2 * G - 1 - LAG
    for n, f in enumerate(EARLY):
        fill[f + 1].update(dict(a=n, b=n - 1) if n else dict(a=n))
    run(0, fill[:G + 1], ORDER_FILL)
    run(0, fill[G + 1:], ORDER)
    out_copy(0, len(EARLY) - 1).start()

    def main(q, _):
        x_copy(q + 2).wait()
        x_copy(q + 3).start()
        steps = [full_step(G - 1 + u) for u in range(G)]
        run(q, steps, ORDER)
        out_copy(q * G + steps[0]["b"], G).start()
    lax.fori_loop(1, NG - 1, main, None)
    x_copy(NG + 1).wait()

    limit = dict(c=H, d=H + G, a=H, b=H)
    drain = [{op: v for op, v in full_step(f).items() if v < limit.get(op, 0)}
             for f in range(H - 1, H + LAG + 1)]
    done = drain[0]["b"]
    for n in (8, 14, 18, 21):
        drain[n]["pre"] = [out_copy(done, drain[n - 1]["b"] - done).start]
        done = drain[n - 1]["b"]
    run(0, drain, ORDER_DRAIN)
    out_copy(done, H - done).start()
    pltpu.make_async_copy(obuf, o_hbm, osem).wait()


@jax.jit
def pallas_standalone__convnext_block__vision_kernel(
    x: jax.Array,
    dw: jax.Array,
    w1: jax.Array,
    w2: jax.Array,
):
    B, H, W, C = x.shape
    assert (B, W, C) == (1, 4 * LANES, 96) and H % G == 0 and H >= 3 * G
    NT = W // LANES
    cslot = -(-G * (C + 1) // 32) * 32
    out = pl.pallas_call(
        _kernel,
        out_shape=jax.ShapeDtypeStruct((H, C, W), x.dtype),
        in_specs=[pl.BlockSpec(memory_space=pl.ANY)] * 4,
        out_specs=pl.BlockSpec(memory_space=pl.ANY),
        scratch_shapes=[
            pltpu.VMEM((XSLOTS * G, C, W), BF16),
            pltpu.VMEM((NT, RSLOTS * C * RPITCH + 32, LANES), U32),
            pltpu.VMEM((C // G, KS * G // 2, W), U32),
            pltpu.VMEM((C * GOUT + 32, LANES), F32),
            pltpu.VMEM((C, 8, W), F32),
            [pltpu.VMEM((RSLOTS * cslot + C, LANES), F32)] * NT,
            pltpu.VMEM((NT, 2 * 4 * C, LANES), F32),
            pltpu.VMEM((H, C, W), BF16),
            pltpu.VMEM((2 * C, LANES), U32),
            pltpu.VMEM((C // 2, 4 * C), U32),
            pltpu.VMEM(dw.shape, BF16),
            pltpu.VMEM(w1.shape, BF16),
            pltpu.VMEM(w1.shape, BF16),
            pltpu.SemaphoreType.DMA((XSLOTS,)),
            pltpu.SemaphoreType.DMA((C // 16,)),
            pltpu.SemaphoreType.DMA(()),
            pltpu.SemaphoreType.DMA((3,)),
        ],
        compiler_params=pltpu.CompilerParams(vmem_limit_bytes=100 * 1024 * 1024),
        name="convnext_block",
    )(jnp.transpose(x, (0, 1, 3, 2)).reshape(H, C, W), dw, w1, w2.T)
    return jnp.transpose(out.reshape(B, H, C, W), (0, 1, 3, 2))
```

```python
import functools

import numpy as np
import jax
import jax.numpy as jnp
from jax import lax
import jax.experimental.pallas as pl
import jax.experimental.pallas.tpu as pltpu

F32, BF16, U32 = jnp.float32, jnp.bfloat16, jnp.uint32

_C1 = float(np.sqrt(2.0 / np.pi))
_ALPHA = float(np.cbrt(_C1 * 0.044715))
_EPS = 1e-5

LANES = 128
KS = 7
G = 16
GOUT = G + 8
XSLOTS = 8
RSLOTS = 4
RPITCH = 9
LAG = 21
X0_SPLIT = (0, 32, 96)
EARLY = (16, 17, 19, 20, 22, 23, 25, 26, 28, 29)

ORDER = ("b0 c0 L0 a0 L1 a1 -d5 -s2 L2 -d4 c1 s1 s0 b1 c2 d0 -s5 r1 r0 -s3 d1 L3 a2 c3 b2 c4 d2 "
         "-f0 s4 c5 g2 d3 a3 g0 g3 g1 f1")
ORDER_FILL = "r0 r1 c0 s0 d0 c1 s1 d1 c2 s2 d2 c3 s3 d3 c4 s4 d4 c5 s5 d5"
ORDER_DRAIN = ORDER


def _dot(a, b):
    return lax.dot_general(a, b, (((1,), (0,)), ((), ())), preferred_element_type=F32)


def _slot(g, n, size):
    v = (g & (n - 1)) * size
    return v if isinstance(v, int) else pl.multiple_of(v, size & -size)


def _tile(k, n=LANES):
    return slice(k * n, (k + 1) * n)


def _kernel(x_hbm, dw_hbm, w1_hbm, w2t_hbm, o_hbm,
            xbuf, rbuf, sbuf, amat, carry, cbuf, gbuf, obuf, w1t, w2t, dwv, w1v, w2v,
            xsem, x0sem, osem, wsem):
    H, C, W = x_hbm.shape
    NT, NG, CP, CPC = W // LANES, H // G, C // 2, C // G
    CPITCH = C + 1
    CSLOT = (cbuf[0].shape[0] - C) // RSLOTS

    def x_copy(g):
        return pltpu.make_async_copy(
            x_hbm.at[pl.ds(jnp.minimum(g, NG - 1) * G, G)],
            xbuf.at[pl.ds(_slot(g, XSLOTS, G), G)], xsem.at[g & (XSLOTS - 1)])

    def x0_copy(m):
        ch = slice(*X0_SPLIT[m:m + 2])
        return pltpu.make_async_copy(x_hbm.at[0:G, ch], xbuf.at[0:G, ch], x0sem.at[m])

    def out_copy(h, n):
        return pltpu.make_async_copy(obuf.at[pl.ds(h, n)], o_hbm.at[pl.ds(h, n)], osem)

    def prepare_weights():
        w1 = jnp.concatenate([w1v[...].astype(F32), jnp.zeros((LANES - C, 4 * C), F32)], axis=0)
        w1t[...] = pltpu.bitcast(w1.T.astype(BF16), U32)
        w2t[...] = pltpu.bitcast(w2v[...], U32)

        spread = jnp.where(lax.broadcasted_iota(jnp.int32, (LANES, LANES), 0)
                           == (lax.broadcasted_iota(jnp.int32, (LANES, LANES), 1) >> 4), 1.0, 0.0)
        taps = []
        for i in range(KS):
            d = jnp.concatenate([dwv[i].astype(F32), jnp.zeros((8 - KS, C), F32)], axis=0)
            d = jnp.concatenate([d, jnp.zeros((8, LANES - C), F32)], axis=1)
            d = jnp.concatenate([d, jnp.zeros((LANES - 8, LANES), F32)], axis=0).T[:C]
            taps.append(_dot(d, spread))
        r = lax.broadcasted_iota(jnp.int32, (C, LANES), 1) & (G - 1)

        def row(rho, _):
            acc = jnp.zeros((C, LANES), F32)
            for i in range(KS):
                acc = jnp.where(r - rho + 7 == i, taps[i], acc)
            amat[pl.ds(rho, C, stride=GOUT), :] = acc
        lax.fori_loop(0, GOUT, row, None)

    def xrow(q, f):
        return _slot(q + (f >> 4), XSLOTS, G) + (f & 15)

    def relayout(q, f, k, c0=0, nc=C):
        a = pltpu.bitcast(xbuf[xrow(q, f), c0:c0 + nc, _tile(k)], U32)
        b = pltpu.bitcast(xbuf[xrow(q, f + 1), c0:c0 + nc, _tile(k)], U32)
        base = _slot(q + (f >> 4), RSLOTS, C * RPITCH) + (c0 // 2 * RPITCH + ((f & 15) >> 1))
        even = (a & np.uint32(0xFFFF)) | (b << 16)
        odd = (a >> 16) | (b & np.uint32(0xFFFF0000))
        rbuf[k, pl.ds(base, nc // 2, stride=RPITCH), :] = even
        rbuf[k, pl.ds(base + CP * RPITCH, nc // 2, stride=RPITCH), :] = odd

    lane = lax.broadcasted_iota(jnp.int32, (8, LANES), 1)

    def shifted(v, d):
        if d == 0:
            return v
        zero = [jnp.zeros((8, LANES), U32)]
        r = [pltpu.roll(t, (-d) % LANES, 1) for t in v]
        own, other = (lane < LANES - d, r[1:] + zero) if d > 0 else (lane >= -d, zero + r[:-1])
        return [jnp.where(own, a, b) for a, b in zip(r, other)]

    def shift(q, f, i):
        c = (f & 15) * CPC + i
        base = _slot(q + (f >> 4), RSLOTS, C * RPITCH) + (c // 2 + CP * (c % 2)) * RPITCH
        v = [rbuf[k, pl.ds(base, 8), :] for k in range(NT)]
        sbuf[i] = jnp.concatenate(
            [jnp.concatenate(shifted(v, j - KS // 2), axis=1) for j in range(KS)], axis=0)

    def conv(f, i):
        c = (f & 15) * CPC + i
        return _dot(amat[_tile(c, GOUT), :][:, :KS * G], pltpu.bitcast(sbuf[i], BF16))

    def conv_store(q, f, i, o):
        g, c = q + (f >> 4), (f & 15) * CPC + i
        if o is None:
            parts = [carry[c]]
        else:
            top = isinstance(g, int) and g == 0
            parts = [o[0:8] if top else o[0:8] + carry[c], o[8:16]]
            carry[c] = o[16:24]
        for k in range(NT):
            for n, p in enumerate(parts):
                rows = pl.ds(_slot(g, RSLOTS, CSLOT) + (8 * n * CPITCH + c), 8, stride=CPITCH)
                cbuf[k][rows, :] = p[:, _tile(k)]

    def layernorm(q, f, k):
        p = f + 4
        y = cbuf[k][pl.ds(_slot(q + (p >> 4), RSLOTS, CSLOT) + (p & 15) * CPITCH, C), :]
        yc = y - jnp.sum(y, axis=0, keepdims=True) * (1.0 / C)
        var = jnp.sum(yc * yc, axis=0, keepdims=True) * (1.0 / C)
        return (yc * (lax.rsqrt(var + _EPS) * _ALPHA)).astype(BF16)

    def expand(h):
        return jnp.concatenate(
            [_dot(pltpu.bitcast(w1t[_tile(j, CP), :], BF16)[:, :C], h) for j in range(4)], axis=0)

    def gelu(f, k, z):
        gbuf[k, _tile(f & 1, 4 * C), :] = z * jnp.tanh(z * (z * z + _C1 / _ALPHA)) + z

    def project(f, k, j):
        g = gbuf[k, pl.ds((f & 1) * 4 * C + j * LANES, LANES), :]
        return _dot(pltpu.bitcast(w2t[:, _tile(j)], BF16), g)

    def residual(q, f, k, o):
        res = xbuf[xrow(q, f), :, _tile(k, 2 * LANES)].astype(F32) + o * (0.5 / _ALPHA)
        obuf[q * G + f, :, _tile(k, 2 * LANES)] = res.astype(BF16)

    def run(q, steps, order):
        vals = [dict() for _ in steps]

        def piece(op, i, st, v):
            if op == "r" and "r" in st:
                relayout(q, st["r"] & ~1, 2 * (st["r"] & 1) + i)
            elif op == "s" and "s" in st:
                shift(q, st["s"], i)
            elif op == "c" and "c" in st:
                v["c", i] = conv(st["c"], i)
            elif op == "d" and "d" in st:
                conv_store(q, st["d"], i, v.get(("c", i)))
            elif op == "L" and "a" in st:
                v["h", i] = layernorm(q, st["a"], i)
            elif op == "a" and "a" in st:
                v["a", i] = expand(v["h", i])
            elif op == "g" and "a" in st:
                gelu(st["a"], i, v["a", i])
            elif op == "b" and "b" in st:
                v["o", i] = project(st["b"], i, 0) + project(st["b"], i, 1) + project(st["b"], i, 2)
                last = project(st["b"], NT - 1, i)
                v["o", NT - 1] = last if i == 0 else v["o", NT - 1] + last
            elif op == "f" and "b" in st:
                residual(q, st["b"], i, jnp.concatenate([v["o", 2 * i], v["o", 2 * i + 1]], axis=1))

        for u in range(len(steps) + 1):
            if u < len(steps):
                for fn in steps[u].get("pre", ()):
                    fn()
            for tok in order.split():
                n = u - 1 if tok[0] == "-" else u
                if 0 <= n < len(steps):
                    piece(tok[-2], int(tok[-1]), steps[n], vals[n])

    def full_step(f):
        return dict(r=f + G + 1, s=f + 1, c=f, d=f, a=f - LAG, b=f - LAG - 1)

    wcopies = [pltpu.make_async_copy(s, d, wsem.at[i])
               for i, (s, d) in enumerate(((dw_hbm, dwv), (w1_hbm, w1v), (w2t_hbm, w2v)))]
    for cp in wcopies:
        cp.start()
    x0_copy(0).start()
    x0_copy(1).start()
    for cp in wcopies:
        cp.wait()
    x_copy(1).start()
    prepare_weights()

    def first_group(m):
        x0_copy(m).wait()
        for f in range(0, G, 2):
            for k in range(NT):
                relayout(0, f, k, X0_SPLIT[m], X0_SPLIT[m + 1] - X0_SPLIT[m])

    fill = [dict(s=0)] + [dict(s=f + 1, c=f, d=f) for f in range(2 * G - 1)]

    def before(f, *fns):
        fill[f + 1].setdefault("pre", []).extend(fns)

    def group(g, f0, nsteps):
        before(f0, x_copy(g).wait, x_copy(g + 1).start)
        for n in range(G // 2):
            before(f0 + n * nsteps // (G // 2),
                   *[functools.partial(relayout, 0, g * G + 2 * n, k) for k in range(NT)])

    before(-1, functools.partial(first_group, 0))
    before(X0_SPLIT[1] // CPC - 1, functools.partial(first_group, 1))
    group(1, 11, 4)
    group(2, 22, 8)
    assert len(EARLY) == 2 * G - 1 - LAG
    for n, f in enumerate(EARLY):
        fill[f + 1].update(dict(a=n, b=n - 1) if n else dict(a=n))
    run(0, fill[:G + 1], ORDER_FILL)
    run(0, fill[G + 1:], ORDER)
    out_copy(0, len(EARLY) - 1).start()

    def main(q, _):
        x_copy(q + 2).wait()
        x_copy(q + 3).start()
        steps = [full_step(G - 1 + u) for u in range(G)]
        run(q, steps, ORDER)
        out_copy(q * G + steps[0]["b"], G).start()
    lax.fori_loop(1, NG - 1, main, None)
    x_copy(NG + 1).wait()

    limit = dict(c=H, d=H + G, a=H, b=H)
    drain = [{op: v for op, v in full_step(f).items() if v < limit.get(op, 0)}
             for f in range(H - 1, H + LAG + 1)]
    done = drain[0]["b"]
    for n in (8, 14, 18, 21):
        drain[n]["pre"] = [out_copy(done, drain[n - 1]["b"] - done).start]
        done = drain[n - 1]["b"]
    run(0, drain, ORDER_DRAIN)
    out_copy(done, H - done).start()
    pltpu.make_async_copy(obuf, o_hbm, osem).wait()


@jax.jit
def pallas_standalone__convnext_block__vision_kernel(
    x: jax.Array,
    dw: jax.Array,
    w1: jax.Array,
    w2: jax.Array,
):
    B, H, W, C = x.shape
    assert (B, W, C) == (1, 4 * LANES, 96) and H % G == 0 and H >= 3 * G
    NT = W // LANES
    cslot = -(-G * (C + 1) // 32) * 32
    out = pl.pallas_call(
        _kernel,
        out_shape=jax.ShapeDtypeStruct((H, C, W), x.dtype),
        in_specs=[pl.BlockSpec(memory_space=pl.ANY)] * 4,
        out_specs=pl.BlockSpec(memory_space=pl.ANY),
        scratch_shapes=[
            pltpu.VMEM((XSLOTS * G, C, W), BF16),
            pltpu.VMEM((NT, RSLOTS * C * RPITCH + 32, LANES), U32),
            pltpu.VMEM((C // G, KS * G // 2, W), U32),
            pltpu.VMEM((C * GOUT + 32, LANES), F32),
            pltpu.VMEM((C, 8, W), F32),
            [pltpu.VMEM((RSLOTS * cslot + C, LANES), F32)] * NT,
            pltpu.VMEM((NT, 2 * 4 * C, LANES), F32),
            pltpu.VMEM((H, C, W), BF16),
            pltpu.VMEM((2 * C, LANES), U32),
            pltpu.VMEM((C // 2, 4 * C), U32),
            pltpu.VMEM(dw.shape, BF16),
            pltpu.VMEM(w1.shape, BF16),
            pltpu.VMEM(w1.shape, BF16),
            pltpu.SemaphoreType.DMA((XSLOTS,)),
            pltpu.SemaphoreType.DMA((2,)),
            pltpu.SemaphoreType.DMA(()),
            pltpu.SemaphoreType.DMA((3,)),
        ],
        compiler_params=pltpu.CompilerParams(vmem_limit_bytes=100 * 1024 * 1024),
        name="convnext_block",
    )(jnp.transpose(x, (0, 1, 3, 2)).reshape(H, C, W), dw, w1, w2.T)
    return jnp.transpose(out.reshape(B, H, C, W), (0, 1, 3, 2))
```

```python
import functools

import numpy as np
import jax
import jax.numpy as jnp
from jax import lax
import jax.experimental.pallas as pl
import jax.experimental.pallas.tpu as pltpu

F32, BF16, U32 = jnp.float32, jnp.bfloat16, jnp.uint32

_C1 = float(np.sqrt(2.0 / np.pi))
_ALPHA = float(np.cbrt(_C1 * 0.044715))
_EPS = 1e-5

LANES = 128
KS = 7
G = 16
GOUT = G + 8
XSLOTS = 8
RSLOTS = 4
RPITCH = 9
LAG = 21
X0_SPLIT = (0, 32, 96)
EARLY = (16, 17, 19, 20, 22, 23, 25, 26, 28, 29)

ORDER_CONV = "c0 s0 d0 c1 s1 d1 c2 s2 d2 c3 s3 d3 c4 s4 d4 c5 s5 d5"
ORDER_FILL = ("-d2 -d3 -g3 -g1 -s5 L3 L1 b0 -d0 c0 -s4 c1 -f0 -f1 L0 a0 b1 b2 -s2 c2 -d5 g0 -s3 s1 c3 "
              "L2 a1 c4 a2 d4 d1 c5 s0 g2 a3")
ORDER_MAIN = ("-d5 b0 r0 c0 b1 c1 r1 -f0 L0 d0 b2 c2 L1 a0 s2 a1 s1 g0 c3 L2 s3 -f1 L3 c4 d3 d1 a2 d4 "
              "s4 s0 g1 g2 a3 d2 g3 c5 s5")
ORDER_DRAIN = "c0 c1 L1 b0 d0 L0 a0 c2 b1 a1 g0 L2 c3 L3 d2 d3 c4 a2 g1 a3 g2 -f0 c5 -d1 -f1 g3 b2 -d4 -d5"


def _dot(a, b):
    return lax.dot_general(a, b, (((1,), (0,)), ((), ())), preferred_element_type=F32)


def _slot(g, n, size):
    v = (g & (n - 1)) * size
    return v if isinstance(v, int) else pl.multiple_of(v, size & -size)


def _tile(k, n=LANES):
    return slice(k * n, (k + 1) * n)


def _kernel(x_hbm, dw_hbm, w1_hbm, w2t_hbm, o_hbm,
            xbuf, rbuf, sbuf, amat, carry, cbuf, gbuf, obuf, w1t, w2t, dwv, w1v, w2v,
            xsem, x0sem, osem, wsem):
    H, C, W = x_hbm.shape
    NT, NG, CP, CPC = W // LANES, H // G, C // 2, C // G
    CPITCH = C + 1
    CSLOT = (cbuf[0].shape[0] - C) // RSLOTS

    def x_copy(g):
        return pltpu.make_async_copy(
            x_hbm.at[pl.ds(jnp.minimum(g, NG - 1) * G, G)],
            xbuf.at[pl.ds(_slot(g, XSLOTS, G), G)], xsem.at[g & (XSLOTS - 1)])

    def x0_copy(m):
        ch = slice(*X0_SPLIT[m:m + 2])
        return pltpu.make_async_copy(x_hbm.at[0:G, ch], xbuf.at[0:G, ch], x0sem.at[m])

    def out_copy(h, n):
        return pltpu.make_async_copy(obuf.at[pl.ds(h, n)], o_hbm.at[pl.ds(h, n)], osem)

    def prepare_weights():
        w1 = jnp.concatenate([w1v[...].astype(F32), jnp.zeros((LANES - C, 4 * C), F32)], axis=0)
        w1t[...] = pltpu.bitcast(w1.T.astype(BF16), U32)
        w2t[...] = pltpu.bitcast(w2v[...], U32)

        spread = jnp.where(lax.broadcasted_iota(jnp.int32, (LANES, LANES), 0)
                           == (lax.broadcasted_iota(jnp.int32, (LANES, LANES), 1) >> 4), 1.0, 0.0)
        taps = []
        for i in range(KS):
            d = jnp.concatenate([dwv[i].astype(F32), jnp.zeros((8 - KS, C), F32)], axis=0)
            d = jnp.concatenate([d, jnp.zeros((8, LANES - C), F32)], axis=1)
            d = jnp.concatenate([d, jnp.zeros((LANES - 8, LANES), F32)], axis=0).T[:C]
            taps.append(_dot(d, spread))
        r = lax.broadcasted_iota(jnp.int32, (C, LANES), 1) & (G - 1)

        def row(rho, _):
            acc = jnp.zeros((C, LANES), F32)
            for i in range(KS):
                acc = jnp.where(r - rho + 7 == i, taps[i], acc)
            amat[pl.ds(rho, C, stride=GOUT), :] = acc
        lax.fori_loop(0, GOUT, row, None)

    def xrow(q, f):
        return _slot(q + (f >> 4), XSLOTS, G) + (f & 15)

    def relayout(q, f, k, c0=0, nc=C):
        a = pltpu.bitcast(xbuf[xrow(q, f), c0:c0 + nc, _tile(k)], U32)
        b = pltpu.bitcast(xbuf[xrow(q, f + 1), c0:c0 + nc, _tile(k)], U32)
        base = _slot(q + (f >> 4), RSLOTS, C * RPITCH) + (c0 // 2 * RPITCH + ((f & 15) >> 1))
        even = (a & np.uint32(0xFFFF)) | (b << 16)
        odd = (a >> 16) | (b & np.uint32(0xFFFF0000))
        rbuf[k, pl.ds(base, nc // 2, stride=RPITCH), :] = even
        rbuf[k, pl.ds(base + CP * RPITCH, nc // 2, stride=RPITCH), :] = odd

    lane = lax.broadcasted_iota(jnp.int32, (8, LANES), 1)

    def shifted(v, d):
        if d == 0:
            return v
        zero = [jnp.zeros((8, LANES), U32)]
        r = [pltpu.roll(t, (-d) % LANES, 1) for t in v]
        own, other = (lane < LANES - d, r[1:] + zero) if d > 0 else (lane >= -d, zero + r[:-1])
        return [jnp.where(own, a, b) for a, b in zip(r, other)]

    def shift(q, f, i):
        c = (f & 15) * CPC + i
        base = _slot(q + (f >> 4), RSLOTS, C * RPITCH) + (c // 2 + CP * (c % 2)) * RPITCH
        v = [rbuf[k, pl.ds(base, 8), :] for k in range(NT)]
        sbuf[i] = jnp.concatenate(
            [jnp.concatenate(shifted(v, j - KS // 2), axis=1) for j in range(KS)], axis=0)

    def conv(f, i):
        c = (f & 15) * CPC + i
        return _dot(amat[_tile(c, GOUT), :][:, :KS * G], pltpu.bitcast(sbuf[i], BF16))

    def conv_store(q, f, i, o):
        g, c = q + (f >> 4), (f & 15) * CPC + i
        if o is None:
            parts = [carry[c]]
        else:
            top = isinstance(g, int) and g == 0
            parts = [o[0:8] if top else o[0:8] + carry[c], o[8:16]]
            carry[c] = o[16:24]
        for k in range(NT):
            for n, p in enumerate(parts):
                rows = pl.ds(_slot(g, RSLOTS, CSLOT) + (8 * n * CPITCH + c), 8, stride=CPITCH)
                cbuf[k][rows, :] = p[:, _tile(k)]

    def layernorm(q, f, k):
        p = f + 4
        y = cbuf[k][pl.ds(_slot(q + (p >> 4), RSLOTS, CSLOT) + (p & 15) * CPITCH, C), :]
        yc = y - jnp.sum(y, axis=0, keepdims=True) * (1.0 / C)
        var = jnp.sum(yc * yc, axis=0, keepdims=True) * (1.0 / C)
        return (yc * (lax.rsqrt(var + _EPS) * _ALPHA)).astype(BF16)

    def expand(h):
        return jnp.concatenate(
            [_dot(pltpu.bitcast(w1t[_tile(j, CP), :], BF16)[:, :C], h) for j in range(4)], axis=0)

    def gelu(f, k, z):
        gbuf[k, _tile(f & 1, 4 * C), :] = z * jnp.tanh(z * (z * z + _C1 / _ALPHA)) + z

    def project(f, k, j):
        g = gbuf[k, pl.ds((f & 1) * 4 * C + j * LANES, LANES), :]
        return _dot(pltpu.bitcast(w2t[:, _tile(j)], BF16), g)

    def residual(q, f, k, o):
        res = xbuf[xrow(q, f), :, _tile(k, 2 * LANES)].astype(F32) + o * (0.5 / _ALPHA)
        obuf[q * G + f, :, _tile(k, 2 * LANES)] = res.astype(BF16)

    def run(q, steps, order):
        vals = [dict() for _ in steps]

        def piece(op, i, st, v):
            if op == "r" and "r" in st:
                relayout(q, st["r"] & ~1, 2 * (st["r"] & 1) + i)
            elif op == "s" and "s" in st:
                shift(q, st["s"], i)
            elif op == "c" and "c" in st:
                v["c", i] = conv(st["c"], i)
            elif op == "d" and "d" in st:
                conv_store(q, st["d"], i, v.get(("c", i)))
            elif op == "L" and "a" in st:
                v["h", i] = layernorm(q, st["a"], i)
            elif op == "a" and "a" in st:
                v["a", i] = expand(v["h", i])
            elif op == "g" and "a" in st:
                gelu(st["a"], i, v["a", i])
            elif op == "b" and "b" in st:
                v["o", i] = project(st["b"], i, 0) + project(st["b"], i, 1) + project(st["b"], i, 2)
                last = project(st["b"], NT - 1, i)
                v["o", NT - 1] = last if i == 0 else v["o", NT - 1] + last
            elif op == "f" and "b" in st:
                residual(q, st["b"], i, jnp.concatenate([v["o", 2 * i], v["o", 2 * i + 1]], axis=1))

        for u in range(len(steps) + 1):
            if u < len(steps):
                for fn in steps[u].get("pre", ()):
                    fn()
            for tok in order.split():
                n = u - 1 if tok[0] == "-" else u
                if 0 <= n < len(steps):
                    piece(tok[-2], int(tok[-1]), steps[n], vals[n])

    def full_step(f):
        return dict(r=f + G + 1, s=f + 1, c=f, d=f, a=f - LAG, b=f - LAG - 1)

    wcopies = [pltpu.make_async_copy(s, d, wsem.at[i])
               for i, (s, d) in enumerate(((dw_hbm, dwv), (w1_hbm, w1v), (w2t_hbm, w2v)))]
    for cp in wcopies:
        cp.start()
    x0_copy(0).start()
    x0_copy(1).start()
    for cp in wcopies:
        cp.wait()
    x_copy(1).start()
    prepare_weights()

    def first_group(m):
        x0_copy(m).wait()
        for f in range(0, G, 2):
            for k in range(NT):
                relayout(0, f, k, X0_SPLIT[m], X0_SPLIT[m + 1] - X0_SPLIT[m])

    fill = [dict(s=0)] + [dict(s=f + 1, c=f, d=f) for f in range(2 * G - 1)]

    def before(f, *fns):
        fill[f + 1].setdefault("pre", []).extend(fns)

    def group(g, f0, nsteps):
        before(f0, x_copy(g).wait, x_copy(g + 1).start)
        for n in range(G // 2):
            before(f0 + n * nsteps // (G // 2),
                   *[functools.partial(relayout, 0, g * G + 2 * n, k) for k in range(NT)])

    before(-1, functools.partial(first_group, 0))
    before(X0_SPLIT[1] // CPC - 1, functools.partial(first_group, 1))
    group(1, 11, 4)
    group(2, 22, 8)
    assert len(EARLY) == 2 * G - 1 - LAG
    for n, f in enumerate(EARLY):
        fill[f + 1].update(dict(a=n, b=n - 1) if n else dict(a=n))
    run(0, fill[:G + 1], ORDER_CONV)
    run(0, fill[G + 1:], ORDER_FILL)
    out_copy(0, len(EARLY) - 1).start()

    def main(q, _):
        x_copy(q + 2).wait()
        x_copy(q + 3).start()
        steps = [full_step(G - 1 + u) for u in range(G)]
        run(q, steps, ORDER_MAIN)
        out_copy(q * G + steps[0]["b"], G).start()
    lax.fori_loop(1, NG - 1, main, None)
    x_copy(NG + 1).wait()

    limit = dict(c=H, d=H + G, a=H, b=H)
    drain = [{op: v for op, v in full_step(f).items() if v < limit.get(op, 0)}
             for f in range(H - 1, H + LAG + 1)]
    done = drain[0]["b"]
    for n in (8, 14, 18, 21):
        drain[n]["pre"] = [out_copy(done, drain[n - 1]["b"] - done).start]
        done = drain[n - 1]["b"]
    run(0, drain, ORDER_DRAIN)
    out_copy(done, H - done).start()
    pltpu.make_async_copy(obuf, o_hbm, osem).wait()


@jax.jit
def pallas_standalone__convnext_block__vision_kernel(
    x: jax.Array,
    dw: jax.Array,
    w1: jax.Array,
    w2: jax.Array,
):
    B, H, W, C = x.shape
    assert (B, W, C) == (1, 4 * LANES, 96) and H % G == 0 and H >= 3 * G
    NT = W // LANES
    cslot = -(-G * (C + 1) // 32) * 32
    out = pl.pallas_call(
        _kernel,
        out_shape=jax.ShapeDtypeStruct((H, C, W), x.dtype),
        in_specs=[pl.BlockSpec(memory_space=pl.ANY)] * 4,
        out_specs=pl.BlockSpec(memory_space=pl.ANY),
        scratch_shapes=[
            pltpu.VMEM((XSLOTS * G, C, W), BF16),
            pltpu.VMEM((NT, RSLOTS * C * RPITCH + 32, LANES), U32),
            pltpu.VMEM((C // G, KS * G // 2, W), U32),
            pltpu.VMEM((C * GOUT + 32, LANES), F32),
            pltpu.VMEM((C, 8, W), F32),
            [pltpu.VMEM((RSLOTS * cslot + C, LANES), F32)] * NT,
            pltpu.VMEM((NT, 2 * 4 * C, LANES), F32),
            pltpu.VMEM((H, C, W), BF16),
            pltpu.VMEM((2 * C, LANES), U32),
            pltpu.VMEM((C // 2, 4 * C), U32),
            pltpu.VMEM(dw.shape, BF16),
            pltpu.VMEM(w1.shape, BF16),
            pltpu.VMEM(w1.shape, BF16),
            pltpu.SemaphoreType.DMA((XSLOTS,)),
            pltpu.SemaphoreType.DMA((2,)),
            pltpu.SemaphoreType.DMA(()),
            pltpu.SemaphoreType.DMA((3,)),
        ],
        compiler_params=pltpu.CompilerParams(vmem_limit_bytes=100 * 1024 * 1024),
        name="convnext_block",
    )(jnp.transpose(x, (0, 1, 3, 2)).reshape(H, C, W), dw, w1, w2.T)
    return jnp.transpose(out.reshape(B, H, C, W), (0, 1, 3, 2))
```
